```python
import os as _os
_os.environ.setdefault("JAX_PLATFORMS", "cpu")
import jax
import jax.numpy as jnp

def _softmax(x, axis=-1):
    return jax.nn.softmax(x, axis=axis)
def _gelu(x):
    return jax.nn.gelu(x, approximate=True)
def _silu(x):
    return jax.nn.silu(x)
def _sigmoid(x):
    return jax.nn.sigmoid(x)
def _layernorm(x, axis=-1, eps=1e-5):
    m = jnp.mean(x, axis=axis, keepdims=True)
    v = jnp.var(x, axis=axis, keepdims=True)
    return (x - m) / jnp.sqrt(v + eps)
def _scatter_add(tgt, idx, src, axis=0):
    return tgt.at[idx].add(src)
def _segment_sum(src, seg, n):
    return jax.ops.segment_sum(src, seg, n)
class _Rng:
    def __init__(self, key):
        self._k = key
    def _next(self):
        self._k, sub = jax.random.split(self._k)
        return sub
    def normal(self, shape):
        return jax.random.normal(self._next(), shape, dtype=jnp.bfloat16)
    def randint(self, lo, hi, shape):
        return jax.random.randint(self._next(), shape, lo, hi, dtype=jnp.int32)
    def uniform(self, shape, lo=0.0, hi=1.0):
        return jax.random.uniform(self._next(), shape, jnp.bfloat16, lo, hi)
    def permutation(self, n):
        return jax.random.permutation(self._next(), n)


kernel_name = 'interleave_layers__spectral_gfnet__mixer_token_mlp__prompt'

def setup_inputs():
    _rng = _Rng(jax.random.key(int.from_bytes(__import__("os").urandom(4), "little")))
    _w = (lambda a: (lambda t: t.astype(jnp.bfloat16) if jnp.issubdtype(t.dtype, jnp.floating) else t)(jnp.asarray(a)))
    def _A_setup():
        B, S, D = 1, 2048, 640
        Df = D // 2 + 1
        return {
            "x": _w((lambda *s: _rng.normal(s) * 0.05)(B, S, D)),
            "w_r": _w((lambda *s: _rng.normal(s) * 0.2)(S, Df) * 0.02),
            "w_i": _w((lambda *s: _rng.normal(s) * 0.2)(S, Df) * 0.02),
        }
    _A_in = _A_setup()

    def _B_setup():
        B, S, D, F = 1, 2048, 640, 1728
        return {
            "x": _w((lambda *s: _rng.normal(s) * 0.05)(B, S, D)),
            "w1": _w((lambda *s: _rng.normal(s) * 0.1)(S, F) * (S ** -0.5)),
            "b1": _w((lambda *s: _rng.normal(s) * 0.1)(F) * 0.02),
            "w2": _w((lambda *s: _rng.normal(s) * 0.1)(F, S) * (F ** -0.5)),
            "b2": _w((lambda *s: _rng.normal(s) * 0.1)(S) * 0.02),
        }
    _B_in = _B_setup()

    return {
        "A_x": _A_in["x"],
        "A_w_r": _A_in["w_r"],
        "A_w_i": _A_in["w_i"],
        "B_x": _B_in["x"],
        "B_w1": _B_in["w1"],
        "B_b1": _B_in["b1"],
        "B_w2": _B_in["w2"],
        "B_b2": _B_in["b2"],
    }

def reference(A_x, A_w_r, A_w_i, B_x, B_w1, B_b1, B_w2, B_b2):
    def _A_ref(x, w_r, w_i):
        B, S, D = x.shape
        X = (lambda x, axes=(-2,-1): jnp.fft.rfft2(x.astype(jnp.float32), axes=axes))(x, axes=(-2, -1))
        W = w_r + 1j * w_i
        X = X * W
        y = (lambda x, s, axes=(-2,-1): jnp.fft.irfft2(x, s=s, axes=axes).astype(jnp.bfloat16))(X, (S, D), axes=(-2, -1))
        return y

    def _B_ref(x, w1, b1, w2, b2):
        B, S, D = x.shape
        h = _layernorm(x, axis=-1)
        u = jnp.einsum("bsd,sf->bdf", h, w1) + b1
        u = _gelu(u)
        y = jnp.einsum("bdf,fs->bds", u, w2) + b2
        return (lambda x, *d: x.transpose(*d))(y, 0, 2, 1)

    x = A_x
    x = x + _A_ref(_layernorm(x, axis=-1), A_w_r, A_w_i)
    x = x + _B_ref(_layernorm(x, axis=-1), B_w1, B_b1, B_w2, B_b2)
    x = x + _A_ref(_layernorm(x, axis=-1), A_w_r, A_w_i)
    x = x + _B_ref(_layernorm(x, axis=-1), B_w1, B_b1, B_w2, B_b2)
    return x
```

```python
import functools

import numpy as np
import jax
import jax.numpy as jnp
import jax.experimental.pallas as pl
import jax.experimental.pallas.tpu as pltpu

S, D, F = 2048, 640, 1728
NB = 16
DH, FH = D // 2, F // 2
DQ, FQ = 160, 384
FR = FH - 2 * FQ
EPS = 1e-5
NBAR = 4
XWAIT = (0, 2, 5, 8, 11, 13)
f32, bf16, u32 = jnp.float32, jnp.bfloat16, jnp.uint32
P = functools.partial

_S1 = np.sin(2 * np.pi / 5)
KAP = float((np.cos(2 * np.pi / 5) - np.cos(4 * np.pi / 5)) / 2)
RHO = float(np.sin(4 * np.pi / 5) / _S1)
TILE_CLASSES = ((0, 5), (1, 9), (2, 8), (7, 3), (6, 4))


def _r5_fwd(y0, y1, y2, y3, y4):
    t1, t2, t3, t4 = y1 + y4, y2 + y3, y1 - y4, y2 - y3
    t5 = t1 + t2
    a = y0 - 0.25 * t5
    b = KAP * (t1 - t2)
    return y0 + t5, a + b, t3 + RHO * t4, a - b, RHO * t3 - t4


def _r5_bwd(y0, r1, i1, r2, i2):
    a = r1 + r2
    b = KAP * (r1 - r2)
    t5 = y0 - 0.25 * a
    t1, t2 = t5 + b, t5 - b
    t3 = i1 + RHO * i2
    t4 = RHO * i1 - i2
    return y0 + a, t1 + t3, t2 + t4, t2 - t4, t1 - t3


def _r10_fwd(x):
    e = [x[(2 * n) % 10] + x[(5 + 2 * n) % 10] for n in range(5)]
    o = [x[(2 * n) % 10] - x[(5 + 2 * n) % 10] for n in range(5)]
    e0, re1, ie1, re2, ie2 = _r5_fwd(*e)
    o0, ro1, io1, ro2, io2 = _r5_fwd(*o)
    return [e0, o0, ro1, io1, re2, ie2, ro2, io2, re1, ie1]


def _r10_bwd(u):
    e0, o0, ro1, io1, re2, ie2, ro2, io2, re1, ie1 = u
    e = _r5_bwd(e0, re1, ie1, re2, ie2)
    o = _r5_bwd(o0, ro1, io1, ro2, io2)
    x = [None] * 10
    for n in range(5):
        x[(2 * n) % 10] = e[n] + o[n]
        x[(5 + 2 * n) % 10] = e[n] - o[n]
    return x


def _barrel(v, where, masks):
    for b in range(4):
        v = [where(masks[b], v[j], v[(j + (1 << b)) % 16]) for j in range(16)]
    return [v[(-k1) % 16] for k1 in range(16)]


@functools.lru_cache(maxsize=None)
def _constants():
    eye = np.eye(D)
    r10 = np.concatenate(_r10_fwd([eye[64 * t:64 * t + 64] for t in range(10)]), axis=0)
    d = np.arange(D)
    rows, scale = [], []
    for cls in TILE_CLASSES:
        for k in cls:
            for u in range(4):
                for part in (0, 1):
                    kd = k + 10 * (8 * u + np.arange(8))
                    kd[kd == 0] = D // 2
                    ang = 2 * np.pi * np.outer(kd, d) / D
                    m = np.cos(ang) if part == 0 else -np.sin(ang)
                    if part == 1:
                        m[kd == D // 2] = 0.0
                    rows.append(m)
                    scale.append(np.where(kd == D // 2, 1.0, 2.0) / (D * S))
    full = np.concatenate(rows, 0) @ np.linalg.inv(r10)
    scale = np.concatenate(scale)
    fwd = [full[128 * t:128 * t + 128, 128 * t:128 * t + 128] for t in range(5)]
    inv = [fwd[t].T * scale[128 * t:128 * t + 128][None, :] for t in range(5)]
    bits = np.stack(fwd + inv).astype(np.float32).astype(jnp.bfloat16).view(np.uint16).astype(np.uint32)
    lmat = bits[:, 0::2, :] | (bits[:, 1::2, :] << 16)
    lane = np.arange(128)
    masks = [(lane & (1 << b)) == 0 for b in range(4)]
    kmap = np.stack(_barrel([np.roll(128 * i + lane, i) for i in range(16)], np.where, masks))
    th = 2 * np.pi * ((np.arange(8)[None, :, None] * kmap[:, None, :]) % S) / S
    th8 = 2 * np.pi * ((8 * kmap) % S) / S
    tab = np.concatenate([np.cos(th).reshape(128, 128), np.sin(th).reshape(128, 128),
                          np.cos(th8), np.sin(th8)], 0).astype(np.float32)
    return lmat, tab


def _dot(a, b):
    return jnp.dot(a, b, preferred_element_type=f32)


def _dot_t(a, b):
    return jax.lax.dot_general(a, b, (((1,), (1,)), ((), ())), preferred_element_type=f32)


def _unpk(x):
    return pltpu.bitcast(x, bf16)


def _pk(x):
    return pltpu.bitcast(x.astype(bf16), u32)


def _cat(xs, axis=0):
    return xs[0] if len(xs) == 1 else jnp.concatenate(xs, axis=axis)


def _cmul_const(re, im, k, n):
    k = k % n
    if k == 0:
        return re, im
    if 4 * k == n:
        return im, -re
    if 4 * k == 3 * n:
        return -im, re
    c, s = float(np.cos(2 * np.pi * k / n)), float(np.sin(2 * np.pi * k / n))
    if (8 * k) % n == 0:
        p, q = re + im, im - re
        if c * s > 0:
            return c * p, c * q
        return (-c) * q, c * p
    return c * re + s * im, c * im - s * re


def _r4_even(z):
    (r0, i0), (r1, i1), (r2, i2), (r3, i3) = z
    ar, ai = r0 + r2, i0 + i2
    cr, ci = r1 + r3, i1 + i3
    return (ar + cr, ai + ci), (ar - cr, ai - ci)


def _r4_odd(z, sign):
    (r0, i0), (r1, i1), (r2, i2), (r3, i3) = z
    br, bi = r0 - r2, i0 - i2
    dr, di = r1 - r3, i1 - i3
    p = (br + di, bi - dr)
    q = (br - di, bi + dr)
    return (p, q) if sign > 0 else (q, p)


def _r4(z, sign):
    o0, o2 = _r4_even(z)
    o1, o3 = _r4_odd(z, sign)
    return [o0, o1, o2, o3]


def _gelu(x):
    t = jnp.tanh(x * (x * x * (0.7978845608028654 * 0.044715) + 0.7978845608028654))
    hx = 0.5 * x
    return hx * t + hx


def _lhs(i, a11, a12, a21, a22):
    return (lambda: a11 + a22, lambda: a21 + a22, lambda: a11, lambda: a22,
            lambda: a11 + a12, lambda: a21 - a11, lambda: a12 - a22)[i]()


def _rhs(i, b11, b12, b21, b22):
    return (lambda: b11 + b22, lambda: b11, lambda: b12 - b22, lambda: b21 - b11,
            lambda: b22, lambda: b11 + b12, lambda: b21 + b22)[i]()


def _comb(m):
    return [m[0] + m[3] - m[4] + m[6], m[2] + m[4], m[1] + m[3], m[0] - m[1] + m[2] + m[5]]


ORDER = (1, 4, 0, 3, 6, 2, 5)
EARLY = (2, 5)
RSUM = {0: 0, 2: 1, 3: 2, 5: 3, 6: 4}
RDEF = {0: (1, (0, 0), (1, 1)), 1: (0, (0, 0)), 2: (-1, (0, 1), (1, 1)), 3: (-1, (1, 0), (0, 0)),
        4: (0, (1, 1)), 5: (1, (0, 0), (0, 1)), 6: (1, (1, 0), (1, 1))}
CMAP = {0: ((0, 0, 1), (1, 1, 1)), 1: ((1, 0, 1), (1, 1, -1)), 2: ((0, 1, 1), (1, 1, 1)),
        3: ((0, 0, 1), (1, 0, 1)), 4: ((0, 0, -1), (0, 1, 1)), 5: ((1, 1, 1),), 6: ((0, 0, 1),)}


def _merge(a, b):
    items = [((k + 0.5) / len(l), n, k) for n, l in enumerate((a, b)) for k in range(len(l))]
    return [(a, b)[n][k] for _, n, k in sorted(items)]


class _Buf:
    def __init__(self, ref, zs, offs, mode):
        self.ref, self.zs, self.offs, self.mode, self.dirty, self.gen = ref, zs, offs, mode, False, 0

    def __setitem__(self, idx, v):
        if len(idx) == 3:
            self.ref.at[idx[0]][idx[1:]] = v
        else:
            self.ref[idx] = v
        self.dirty = True

    def __getitem__(self, key):
        ref = self.ref
        if self.mode == "D":
            if self.dirty:
                self.dirty = False
                self.gen = (self.gen + 1) % 8
            at = (self.gen, key[0].start)
            if at not in self.offs:
                self.offs[at] = pl.multiple_of(self.zs[self.gen] + key[0].start, 8)
            return ref[pl.ds(self.offs[at], key[0].size), key[1]]
        if self.dirty:
            self.dirty = False
            if len(ref.shape) == 3 and ref.shape[0] > 8:
                idx = (self.zs[0] + ref.shape[0] - 1, pl.ds(0, 8))
            else:
                row = pl.ds(pl.multiple_of(self.zs[0] + ref.shape[-2] - 8, 8), 8)
                idx = (0,) * (len(ref.shape) - 2) + (row,)
            ref[idx + (pl.ds(0, 128),)] = jnp.zeros((8, 128), ref.dtype)
        return ref[key]

    def touch(self):
        if self.mode != "N":
            self.dirty = True


class _Rows:
    def __init__(self, buf):
        self.buf = buf

    @staticmethod
    def _split(r0, n):
        while n:
            k = min(n, 64 - r0 % 64)
            yield r0 + 8 * (r0 // 64), k
            r0, n = r0 + k, n - k

    def ld(self, r0, n, fresh=True):
        src = self.buf if fresh else self.buf.ref
        return _cat([src[pl.ds(p, k), slice(None)] for p, k in self._split(r0, n)])

    def st(self, r0, v):
        o = 0
        for p, k in self._split(r0, v.shape[0]):
            self.buf[pl.ds(p, k), slice(None)] = v if k == v.shape[0] else v[o:o + k]
            o += k

    def touch(self):
        self.buf.touch()


def _kernel(z_hbm, x_hbm, wr_hbm, wi_hbm, w1_hbm, b1_hbm, w2_hbm, b2_hbm, lm_hbm, tab_hbm, out_hbm,
            xin, wraw, w1v, w2v, b1v, b2v, lm, tab, Y, ACC, MEAN, barv, z_ref, sem,
            cs, W, X, TB, ZB, LA, LAE, LAQ, S1, S1X, S1R, S1Q, S2, S2R, LG, LGR):
    zs, offs = [], {}
    wrap = lambda t, m: [wrap(v, m) for v in t] if isinstance(t, (list, tuple)) else _Buf(t, zs, offs, m)
    X = [_Rows(b) for b in wrap(X, "D")]
    W, TB, ZB, S1, S1X, S1R, S2, S2R = wrap([W, TB, ZB, S1, S1X, S1R, S2, S2R], "F")
    cs, LA, LAE, LAQ, S1Q, LG, LGR = wrap([cs, LA, LAE, LAQ, S1Q, LG, LGR], "N")
    outv = xin

    mk = pltpu.make_async_copy
    order16 = [a + 4 * c for a in range(4) for c in range(4)]
    xsem = [max(i for i, w in enumerate(XWAIT) if w <= n) for n in range(NB)]
    cp_x = [mk(x_hbm.at[0, pl.ds(128 * al, 128), :], xin.at[al], sem.at[xsem[n]]) for n, al in enumerate(order16)]
    cp_z = mk(z_hbm, z_ref, sem.at[6])
    cp_tab = mk(tab_hbm, tab, sem.at[7])
    cp_l = mk(lm_hbm.at[pl.ds(0, 5)], lm.at[pl.ds(0, 5)], sem.at[8])
    cp_li = mk(lm_hbm.at[pl.ds(5, 5)], lm.at[pl.ds(5, 5)], sem.at[9])
    cp_b = [mk(b1_hbm, b1v, sem.at[10]), mk(b2_hbm, b2v, sem.at[10])]
    cp_w = [[mk(src.at[pl.ds(80 * q, 80), :], wraw.at[p, pl.ds(80 * q, 80), :], sem.at[11 + h])
             for q in (2 * h, 2 * h + 1) for p, src in enumerate((wr_hbm, wi_hbm))] for h in range(2)]
    cp_w[0][2:2] = [mk(src.at[pl.ds(320, 1), :], wraw.at[p, pl.ds(320, 1), :], sem.at[11])
                    for p, src in enumerate((wr_hbm, wi_hbm))]
    cols = lambda src, dst, c, s: mk(src.at[:, pl.ds(128 * c, 128)], dst.at[c], sem.at[s])
    cp_w1 = [[cols(w1_hbm, w1v, 4 * c, 13) for c in range(4)],
             [cols(w1_hbm, w1v, 4 * c + 1, 14) for c in range(4)],
             [cols(w1_hbm, w1v, 4 * c + a, 15) for a in (2, 3) for c in range(4)]]
    cp_w2 = [cols(w2_hbm, w2v, c, 16) for c in range(NB)]
    SEM_OUT = 17
    bars = [mk(tab_hbm.at[pl.ds(0, 8), :], barv.at[i], sem.at[18 + i]) for i in range(NBAR)]

    def start(cps, prio):
        for c in cps:
            c.start(priority=prio)

    def wait(cps):
        for c in cps:
            c.wait()

    start([cp_tab, cp_l, cp_z] + cp_b + bars, 0)
    start(cp_x, 1)
    cp_tab.wait()

    ACC[:, :, pl.ds(2 * FQ, 128)] = jnp.zeros((7, DH, 128), f32)
    for k1 in range(16):
        c = tab[pl.ds(8 * k1, 8), :]
        s = tab[pl.ds(128 + 8 * k1, 8), :]
        c8 = jnp.broadcast_to(tab[pl.ds(256 + k1, 1), :], (8, 128))
        s8 = jnp.broadcast_to(tab[pl.ds(272 + k1, 1), :], (8, 128))
        prev = None
        for v in range(16):
            cur = (c, s - c, c + s)
            if v % 2:
                for x in range(3):
                    cs[pl.ds(8 * (v // 2), 8), pl.ds(128 * (3 * k1 + x), 128)] = _pk(_cat([prev[x], cur[x]]))
            prev = cur
            if v < 15:
                c, s = c * c8 - s * s8, s * c8 + c * s8
    cp_l.wait()
    cp_z.wait()
    zs.extend(z_ref[g] for g in range(8))

    never = jnp.full((8, 128), zs[0], jnp.int32).astype(u32) != 0
    side = []
    rate = [0.0, 0.0]

    def feed(pieces, ndots, delay=0.0):
        assert not side
        side.extend(pieces)
        rate[0] = len(pieces) / float(ndots)
        rate[1] = -delay * rate[0]

    def run(pieces):
        for f in pieces:
            f()

    def flush():
        while side:
            side.pop(0)()

    def dep(x):
        rate[1] += rate[0]
        k = min(max(int(rate[1] + 1e-6), 0), len(side))
        rate[1] -= k
        toks = [t for t in [side.pop(0)() for _ in range(k)] if t is not None]
        if not toks:
            return x
        nv = x.shape[0] // 8
        col = x[:, :128] if x.shape[1] > 128 else x
        at = {}
        for n, t in enumerate(toks):
            at.setdefault((n * nv) // len(toks), []).append(t)
        segs, pos = [], 0
        for i, ts in at.items():
            if i > pos:
                segs.append(col[8 * pos:8 * i])
            head = col[8 * i:8 * i + 8]
            for t in ts:
                t = t if t.shape[0] == 8 else t[:8]
                head = jax.lax.select(never, t if t.dtype == u32 else pltpu.bitcast(t, u32), head)
            segs.append(head)
            pos = i + 1
        if pos < nv:
            segs.append(col[8 * pos:])
        return _cat(segs) if x.shape[1] == 128 else _cat([_cat(segs), x[:, 128:]], 1)

    def freq_rows(k, u):
        return pl.ds(80 * u + k // 2 + 40 * (k % 2), 8, stride=5)

    def xpose_in(al):
        row = jax.lax.broadcasted_iota(jnp.int32, (128, 128), 0)
        col = jax.lax.broadcasted_iota(jnp.int32, (128, 128), 1)
        eye = _pk(jnp.where(row == col, 1.0, 0.0))
        for t in range(5):
            X[al].st(128 * t, _dot_t(_unpk(dep(eye)), xin[al, :, pl.ds(128 * t, 128)]))

    def front_block(al, rstd):
        a, c = al % 4, al // 4
        acc, e0, held = [None, None, None], [], {}

        def chunk(u):
            us = _r10_fwd([X[al].ld(64 * t + 8 * u, 8) for t in range(10)])
            e0.append(us[0])
            for t in range(1, 10):
                g = 0 if t == 1 else (1 if t % 2 == 0 else 2)
                sq = us[t] * us[t]
                acc[g] = sq if acc[g] is None else acc[g] + sq
                if u % 2:
                    TB[a][pl.ds(32 * t + 4 * (u - 1), 8), pl.ds(128 * c, 128)] = _pk(_cat([held[t], us[t]]))
                held[t] = us[t]
            return acc[2]

        def fin():
            m10 = jnp.sum(sum(e0[1:], e0[0]), axis=0, keepdims=True) * (1.0 / 64.0)
            MEAN[pl.ds(al, 1), :] = m10 * 0.1
            e = [v - m10 for v in e0]
            TB[a][pl.ds(0, 32), pl.ds(128 * c, 128)] = _pk(_cat(e))
            a0 = sum((v * v for v in e), acc[0])
            tot = a0 * 0.1 + acc[1] * 0.2 + acc[2] * float(_S1 * _S1 / 5.0)
            var = jnp.sum(tot, axis=0, keepdims=True) * (1.0 / D)
            rstd[c] = jax.lax.rsqrt(var + EPS)
            return tot
        return [P(chunk, u) for u in range(8)] + [fin]

    def front_group(a, rstd, ts=range(5)):
        for t in ts:
            z = _dot(_unpk(dep(lm[t])), _unpk(TB[a][pl.ds(64 * t, 64), :]))
            z = [z[:, 128 * c:128 * c + 128] * rstd[c] for c in range(4)]
            s02, s13, d02, d13 = z[0] + z[2], z[1] + z[3], z[0] - z[2], z[1] - z[3]
            o0, o2 = s02 + s13, s02 - s13
            for h, k in enumerate(TILE_CLASSES[t]):
                for u in range(4):
                    r0 = 64 * h + 16 * u
                    y0, y2, (br, bi), (dr, di) = [(v[r0:r0 + 8], v[r0 + 8:r0 + 16]) for v in (o0, o2, d02, d13)]
                    for j, y in enumerate((y0, (br + di, bi - dr), y2, (br - di, bi + dr))):
                        re, im = _cmul_const(y[0], y[1], a * j, 16)
                        Y[(a * 4 + j) * 2, freq_rows(k, u), :] = re
                        Y[(a * 4 + j) * 2 + 1, freq_rows(k, u), :] = im

    def wprep(q):
        lane = jax.lax.broadcasted_iota(jnp.int32, (8, 128), 1)
        sub = jax.lax.broadcasted_iota(jnp.int32, (8, 128), 0)
        masks = [(lane & (1 << b)) == 0 for b in range(4)]
        nets = [(g, p) for g in range(5 * q, 5 * q + 5) for p in range(2)]
        state = {}

        def rolls(n):
            g, p = nets[n]
            v = []
            for i in range(16):
                x = pltpu.bitcast(wraw[p, pl.ds(16 * g, 16), pl.ds(128 * i, 128)], u32)
                if g == 0:
                    ny = wraw[p, pl.ds(320, 1), pl.ds(128 * i, 128)].astype(f32)
                    nyb = pltpu.bitcast(jnp.broadcast_to(ny, (8, 128)), u32) >> 16
                    x = jnp.where(sub == 0, (x & jnp.uint32(0xFFFF0000)) | nyb, x)
                v.append(pltpu.roll(x, i, 1) if i else x)
            state[n] = v

        def sel(n):
            g, p = nets[n]
            v = _barrel(state.pop(n), jax.lax.select, masks)
            for k1 in range(16):
                W[q][2 * k1 + p, pl.ds(8 * (g % 5), 8), :] = v[k1]
            return v[15]
        return [f for n in range(13) for f in [P(rolls, n)][:n < 10] + [P(sel, n - 3)][:n >= 3]]

    def wload(k1, p, r0):
        x = [W[q][2 * k1 + p, pl.ds(0, 40), :] for q in (r0 // 80, r0 // 80 + 1)]
        return pltpu.bitcast(_cat([y for v in x for y in (v << 16, v & jnp.uint32(0xFFFF0000))]), f32)

    def mid(hooks=None):
        staged = hooks is not None
        pre, part = {}, {}
        for t in W:
            t.touch()

        def fwd(un, i):
            j, r0, m = un
            k1 = j + 4 * m
            if (j, r0, m % 2) not in pre:
                z = [(Y[(a * 4 + j) * 2, pl.ds(r0, DQ), :], Y[(a * 4 + j) * 2 + 1, pl.ds(r0, DQ), :])
                     for a in range(4)]
                pre[j, r0, m % 2] = [[v.astype(bf16) for v in (re + im, im, re)]
                                     for re, im in (_r4_odd(z, +1) if m % 2 else _r4_even(z))]
            t = part.setdefault(("t", un), {})
            t[i] = _dot(pre[j, r0, m % 2][m // 2][i],
                        _unpk(dep(cs[pl.ds(0, 64), pl.ds(128 * (3 * k1 + i), 128)])))
            if len(t) == 3:
                part["x", un] = (t[0] + t[1], t[0] - t[2])
                if staged:
                    for x in range(2):
                        ZB[k1 // 4][k1 % 4, pl.ds(328 * x + r0, DQ), :] = part["x", un][x]

        def inv(un, i):
            j, r0, m = un
            k1 = j + 4 * m
            if ("y", un) not in part:
                t = part.pop(("x", un))
                if staged:
                    t = [ZB[k1 // 4][k1 % 4, pl.ds(328 * x + r0, DQ), :] for x in range(2)]
                wr, wi = wload(k1, 0, r0), wload(k1, 1, r0)
                yr = t[0] * wr - t[1] * wi
                yi = t[0] * wi + t[1] * wr
                part["y", un] = [v.astype(bf16) for v in (yr + yi, yi, yr)]
            q = part.setdefault(("q", un), {})
            q[i] = _dot_t(part["y", un][i],
                          _unpk(dep(cs[pl.ds(0, 64), pl.ds(128 * (3 * k1 + (0, 2, 1)[i]), 128)])))
            qs = [part.get(("q", (j, r0, mm)), ()) for mm in range(4)]
            if all(len(x) == 3 for x in qs):
                y = _r4([(x[0] - x[1], x[0] + x[2]) for x in qs], -1)
                for a in range(4):
                    Y[(a * 4 + j) * 2, pl.ds(r0, DQ), :] = y[a][0]
                    Y[(a * 4 + j) * 2 + 1, pl.ds(r0, DQ), :] = y[a][1]

        quads = [(j, r0) for r0 in (0, DQ) for j in range(4)]
        if staged:
            for f in (fwd, inv):
                for n, (j, r0) in enumerate(quads):
                    run(hooks.get((f is inv, n), ()))
                    for i, m in enumerate((0, 1, 3)):
                        run([P(f, (j, r0, m), x) for x in range(3)] + [P(f, (j, r0, 2), i)])
        else:
            for j, r0 in quads:
                for n, m in enumerate((0, 0, 1, 1, 3, 3)):
                    run([P((fwd, inv)[n % 2], (j, r0, m), x) for x in range(3)])
                    (fwd, inv)[n // 3]((j, r0, 2), n % 3)

    def back_group(a, ts=range(5)):
        for t in ts:
            y = [_cmul_const(*[_cat([Y[(a * 4 + j) * 2 + x, freq_rows(k, u), :]
                                     for k in TILE_CLASSES[t] for u in range(4)]) for x in range(2)], -a * j, 16)
                 for j in range(4)]
            rhs = _cat([_cat([v[r:r + 8] for r in range(0, 64, 8) for v in z]) for z in _r4(y, -1)], 1).astype(bf16)
            z = _dot(_unpk(dep(lm[5 + t])), rhs)
            for c in range(4):
                for h in range(2):
                    ZB[a][c, pl.ds(72 * (2 * t + h), 64), :] = z[64 * h:64 * h + 64, 128 * c:128 * c + 128]

    def back_block(a, c, st):
        al = a + 4 * c
        acc = [None, None, None]

        def chunk(u):
            if u == 0:
                acc[2] = jnp.broadcast_to(MEAN[pl.ds(al, 1), :], (8, 128))
            ys = _r10_bwd([ZB[a][c, pl.ds(72 * t + 8 * u, 8), :] for t in range(10)])
            for t in range(10):
                xn = X[al].ld(64 * t + 8 * u, 8, False) + ys[t]
                X[al].st(64 * t + 8 * u, xn)
                xc = xn - acc[2]
                acc[0] = xc if acc[0] is None else acc[0] + xc
                acc[1] = xc * xc if acc[1] is None else acc[1] + xc * xc
            return acc[1]

        def fin():
            dm = jnp.sum(acc[0], axis=0, keepdims=True) * (1.0 / D)
            var = jnp.sum(acc[1], axis=0, keepdims=True) * (1.0 / D) - dm * dm
            r = jax.lax.rsqrt(var + EPS)
            r = r * jax.lax.rsqrt(var * r * r + EPS)
            st[c] = (jnp.broadcast_to(acc[2][:1] + dm, (16, 128)), jnp.broadcast_to(r, (16, 128)))
            return st[c][1]
        return [P(chunk, u) for u in range(8)] + [fin]

    def normed(a, c, st, r0):
        return (X[a + 4 * c].ld(r0, 16) - st[c][0]) * st[c][1]

    def norm_pair(a, p, st, which):
        def chunk(u):
            if u == 0:
                X[a + 4 * p].touch()
            a11, a21 = normed(a, p, st, 16 * u), normed(a, p, st, DH + 16 * u)
            a12 = a22 = None
            if which != EARLY:
                a12, a22 = normed(a, p + 2, st, 16 * u), normed(a, p + 2, st, DH + 16 * u)
            for i in which:
                v = _lhs(i, a11, a12, a21, a22)
                if which == EARLY:
                    LAE[p][pl.ds(8 * u, 8), pl.ds(128 * EARLY.index(i), 128)] = _pk(v)
                else:
                    LA[a][i, pl.ds(8 * u, 8), pl.ds(128 * p, 128)] = _pk(v)
            return v
        return [P(chunk, u) for u in range(DH // 16)]

    def norm_quad(a, st):
        h = {}

        def load(u, rq):
            for c in range(4):
                h[rq, c] = normed(a, c, st, DQ * rq + 16 * u)
            return h[rq, 3]

        def outs(u, i):
            l1 = [_lhs(i, h[rq, p], h[rq, p + 2], h[rq + 2, p], h[rq + 2, p + 2])
                  for rq in range(2) for p in range(2)]
            for x in range(4):
                LA[a][i, pl.ds(DQ // 2 * (x // 2) + 8 * u, 8), pl.ds(128 * (x % 2), 128)] = _pk(l1[x])
            for k in (0, 1, 4, 5, 6):
                v = _lhs(k, *l1)
                LAQ[7 * i + k, pl.ds(8 * u, 8), pl.ds(128 * (a - 2), 128)] = _pk(v)
            return v
        return [f for u in range(DQ // 16)
                for f in [P(load, u, rq) for rq in range(4)] + [P(outs, u, i) for i in range(7)]]

    zsum = {}

    def wblock(src, a, kh, nh, k2, n2, r0, z):
        f1, s1, f2, s2 = (nh, kh, n2, k2) if src is w1v else (kh, nh, k2, n2)
        blk = a + 4 * s2 + 8 * s1
        if z is not None:
            if (z, blk) not in zsum:
                zsum[z, blk] = zs[z] + blk
            blk = zsum[z, blk]
        return src[blk, pl.ds(FH * f1 + FQ * f2 + r0, 16), :].astype(f32)

    def wsum(src, dst, a, lo, which=tuple(RSUM), z=None):
        def pos(r0, p):
            k2, n2 = (p, 0) if src is w1v else (0, p)
            used = {b for i in which for b in RDEF[i][1:]}
            q = [wblock(src, a, kh, nh, k2, n2, r0, z) if (kh, nh) in used else None
                 for kh in range(2) for nh in range(2)]
            buf = dst if lo else dst[r0 // 128]
            for i in which:
                v = _rhs(i, *q)
                buf[RSUM[i], pl.ds(r0 % 128 // 2, 8), pl.ds(128 * p, 128)] = _pk(v)
            return v
        return [P(pos, r0, p) for r0 in range(lo, FH, 16) for p in range(2)]

    def wpos2(src, a, i, r0, dst):
        sg, *ops = RDEF[i]
        l1 = []
        for k2 in range(2):
            for n2 in range(2):
                x = [wblock(src, a, kh, nh, k2, n2, r0, i) for kh, nh in ops]
                l1.append(x[0] if sg == 0 else x[0] + x[1] if sg > 0 else x[0] - x[1])
        tok = None
        for k in range(7):
            v = _rhs(k, *l1)
            if i in RSUM or k in RSUM:
                buf, idx = dst(k)
                buf[idx] = _pk(v)
            if k in RSUM:
                h = pltpu.bitcast(v[8 * (k % 2):8 * (k % 2) + 8], u32)
                tok = h if tok is None else tok | h
        return tok

    def wsum1q(ci):
        return [P(wpos2, w1v, a, i, 128 * ci + r0,
                  lambda k, a=a, i=i, r0=r0: (S1Q[ci], (7 * i + k, pl.ds(r0 // 2, 8), pl.ds(128 * (a - 2), 128))))
                for i in ORDER for a in (2, 3) for r0 in range(0, 128, 16)]

    def wsum2(a, n):
        i = ORDER[n]
        return ([P(wpos2, w2v, a, i, r0, lambda k, r0=r0: (S2[a][i], (pl.ds(r0 // 2, 8), pl.ds(128 * k, 128))))
                 for r0 in range(0, FQ, 16)] + (wsum(w2v, S2R[a], a, 2 * FQ) if n == 1 else []))

    def mm1(gs, i, n0, ps, first):
        n = min(128, FH - n0)
        lanes = pl.ds(128 * ps[0], 128 * len(ps))
        lhs, rhs = [], []
        for a in gs:
            if a == 0 and i in EARLY:
                lhs += [LAE[p][pl.ds(0, DH // 2), pl.ds(128 * EARLY.index(i), 128)] for p in ps]
            else:
                lhs.append(LA[a][i, pl.ds(0, DH // 2), lanes])
        for a in gs:
            if i in RSUM:
                buf = S1R[a - 2] if a >= 2 else (S1X if a == 0 and i not in EARLY else S1[a])[n0 // 128]
                rhs.append(_unpk(buf[RSUM[i], pl.ds(0, n // 2), lanes]))
            else:
                hf = 0 if i == 1 else 1
                rhs.append(_cat([w1v[a + 4 * p + 8 * hf, pl.ds(FH * hf + n0, n), :] for p in ps], 1))
        r = _dot_t(_unpk(dep(_cat(lhs, 1))), _cat(rhs, 1))
        if not first:
            r = ACC[i, :, pl.ds(n0, n)] + r
        elif i in (2, 3):
            off = n0 + (FH if i == 2 else 0)
            r = r + b1v[...].astype(f32).reshape(1, F)[:, off:off + n]
        ACC[i, :, pl.ds(n0, n)] = r

    def mm1_pair(ci):
        for i in ORDER:
            hf = 0 if i == 1 else 1
            m = {}
            for k in ORDER:
                if k in (2, 3):
                    lhs = _cat([LA[a][i, pl.ds(DQ // 2 * (k - 2), DQ // 2), pl.ds(128 * (k - 2), 128)]
                                for a in (2, 3)], 1)
                else:
                    lhs = LAQ[7 * i + k, pl.ds(0, DQ // 2), :]
                if i in RSUM or k in RSUM:
                    rhs = _unpk(S1Q[ci][7 * i + k, pl.ds(0, 64), :])
                else:
                    h2 = 0 if k == 1 else 1
                    rhs = _cat([w1v[a + 4 * h2 + 8 * hf, pl.ds(FH * hf + FQ * h2 + 128 * ci, 128), :]
                                for a in (2, 3)], 1)
                m[k] = _dot_t(_unpk(dep(lhs)), rhs)
            for x, c in enumerate(_comb(m)):
                idx = (i, pl.ds(DQ * (x // 2), DQ), pl.ds(128 * ci + FQ * (x % 2), 128))
                ACC[idx] = ACC[idx] + c
        flush()

    def gelu4(r0, n0):
        return [_gelu(c) for c in _comb([ACC[i, pl.ds(r0, 16), pl.ds(n0, 128)] for i in range(7)])]

    def gelu_rem():
        def piece(r0):
            g = gelu4(r0, 2 * FQ)
            for i in range(7):
                v = _lhs(i, *g)
                LGR[pl.ds(r0 // 2, 8), pl.ds(128 * i, 128)] = _pk(v)
            return v
        return [P(piece, r0) for r0 in range(0, DH, 16)]

    def gelu_pair(n0):
        g = {}

        def quad(r0, x):
            g[x] = gelu4(r0 + DQ * (x // 2), n0 + FQ * (x % 2))
            return g[x][3]

        def outs(r0, i):
            l1 = [_lhs(i, *g[x]) for x in range(4)]
            for k in range(7):
                v = _lhs(k, *l1)
                LG[7 * i + k, pl.ds(r0 // 2, 8), pl.ds(n0, 128)] = _pk(v)
            return v
        return [f for r0 in range(0, DQ, 16)
                for f in [P(quad, r0, x) for x in range(4)] + [P(outs, r0, i) for i in range(7)]]

    def back_mm1(layer, wait_a, wait_b, wait_c):
        new = layer == 0
        for t in S1X + S1[0] + S1[1] + S1R:
            t.touch()
        st = {}
        late = (0, 1, 3, 4, 6)
        we = wsum(w1v, S1[0], 0, 0, EARLY) if new else []
        wl = wsum(w1v, S1X, 0, 0, (0, 3, 6), 7) if new else []
        wq = [wsum1q(ci) if new else [] for ci in range(3)]
        back_group(0)
        back_group(1, (0,))
        feed(_merge(back_block(0, 0, st) + norm_pair(0, 0, st, EARLY) + back_block(0, 1, st), we[0::2]), 14)
        back_group(1, (1, 2, 3, 4))
        back_group(2)
        back_group(3)

        def work(a):
            nst = {}
            if a >= 2:
                return sum([back_block(a, c, nst) for c in range(4)], []) + norm_quad(a, nst)
            return sum([back_block(a, p, nst) + back_block(a, p + 2, nst) + norm_pair(a, p, nst, range(7))
                        for p in range(2)], [])

        chunks = range(0, 2 * FQ + (128 if new else 0), 128)
        slots = [(0, i, n0, (p,), p == 0) for p in range(2) for i in EARLY[::-1] for n0 in chunks]
        e1, e2 = len(slots) // 2, len(slots)
        slots += [(0, i, n0, (0, 1), True) for i in ORDER[:5] for n0 in chunks]
        e3 = len(slots) - (6 if new else 8)
        slots += [(1, i, n0, (0, 1), False) for i in ORDER for n0 in chunks]
        for si, (a, i, n0, ps, first) in enumerate(slots):
            if si in (0, e1, e2, e3):
                flush()
            if si == 0:
                feed(_merge(norm_pair(0, 1, st, EARLY) + back_block(0, 2, st), we[1::2] + wl[:27]), e1 - 1)
            if si == e1:
                feed(_merge(back_block(0, 3, st) + norm_pair(0, 0, st, late), wl[27:]), e1 - 1)
            if si == e2:
                run(norm_pair(0, 1, st, late))
                wait_a()
                feed(_merge(work(1), wsum(w1v, S1[1], 1, 0) if new else []), e3 - e2 - 1)
            if si == e3:
                wait_b()
                feed(_merge(work(2) + work(3), wq[0]), len(slots) - e3 - 1)
            mm1((a,), i, n0, ps, first)
        flush()
        feed(wq[1] + (wsum(w1v, S1R[0], 2, 2 * FQ) + wsum(w1v, S1R[1], 3, 2 * FQ) if new else []), 48)
        mm1_pair(0)
        feed(_merge(gelu_pair(0), wq[2]), 48)
        mm1_pair(1)
        wait_c()
        feed(_merge(gelu_pair(128), wsum2(0, 0) if new else []), 48)
        mm1_pair(2)
        feed(gelu_pair(256), 6.0, 0.5 if new else 0.3)
        for i in ORDER:
            mm1((2, 3) if new else (0, 1, 2, 3), i, 2 * FQ, (0, 1), not new)
        flush()
        return gelu_rem()

    def mm2_group(a, done, plan, top=None):
        b2 = b2v[...].astype(f32)
        for t in [S2R[a]] + S2[a] + [X[a + 4 * c] for c in range(4)]:
            t.touch()
        q = {(rq, c): X[a + 4 * c].ld(DQ * rq, DQ, False) + b2[a + 4 * c:a + 4 * c + 1]
             for rq in range(4) for c in range(4)}
        for n, i in enumerate(ORDER):
            run(plan.get(n, ()))
            hf = 0 if i == 1 else 1
            m = {}
            for k in ORDER:
                lhs = _unpk(dep(LG[7 * i + k, pl.ds(0, DQ // 2), :]))
                if i in RSUM or k in RSUM:
                    rhs = _unpk(S2[a][i][pl.ds(0, FQ // 2), pl.ds(128 * k, 128)])
                else:
                    h2 = 0 if k == 1 else 1
                    rhs = w2v[a + 4 * h2 + 8 * hf, pl.ds(FH * hf + FQ * h2, FQ), :]
                m[k] = _dot(lhs, rhs)
                if k == (5 if a == n == 0 else 6):
                    if a == n == 0:
                        flush()
                    if i in RSUM:
                        rhs = _unpk(S2R[a][RSUM[i], pl.ds(0, FR // 2), :])
                    else:
                        rhs = _cat([w2v[a + 4 * p + 8 * hf, pl.ds(FH * hf + 2 * FQ, FR), :] for p in range(2)], 1)
                    r = _dot(_unpk(LGR[pl.ds(0, DH // 2), pl.ds(128 * i, FR)]), rhs)
            for x, c in enumerate(_comb(m)):
                rq, p = x // 2, x % 2
                c = c + r[DQ * rq:DQ * rq + DQ, 128 * p:128 * p + 128]
                for rh, ch, sg in CMAP[i]:
                    key = (2 * rh + rq, 2 * ch + p)
                    q[key] = q[key] + c if sg > 0 else q[key] - c
            if n == 5 and top is not None:
                for c in (2, 3):
                    top(a + 4 * c, [q[rq, c] for rq in range(2)])
            for c in {4: (0, 1), 6: (2, 3)}.get(n, ()):
                done(a + 4 * c, [q[rq, c] for rq in range(4)])

    def mm2_front(carry):
        pend = prev = None
        for a in range(4):
            rstd, new, fbq = {}, [], []

            def done(al, parts):
                for rq in range(4):
                    X[al].st(DQ * rq, parts[rq])
                new.extend(front_block(al, rstd))

            def step(n):
                flush()
                nxt = 7 * a + n + 1
                w = wsum2(nxt // 7, nxt % 7) if nxt < 28 else []
                if n == 0:
                    fbq.extend(carry)
                if n == 5:
                    fbq.extend(new)
                    new.clear()
                nd = 6 + (1 if 0 < a < 3 and n >= 2 else 0)
                lag = 4 if n in (0, 5) and (a, n) != (0, 0) else 0
                fb = fbq[:len(fbq) // 4] if lag else list(fbq)
                del fbq[:len(fb)]
                k = int(len(w) * lag / nd)
                if w:
                    feed(w[:k] + _merge(w[k:], fb), nd)
                elif fb:
                    feed(fb, nd - lag, lag)

            plan = {n: [P(step, n)] for n in range(7)}
            if 0 < a < 3:
                for t in range(5):
                    plan[2 + t].append(P(front_group, pend[0], pend[1], (t,)))
            mm2_group(a, done, plan)
            flush()
            carry = new
            prev, pend = pend, (a, rstd)
        feed(carry, 3, 2)
        front_group(*prev)
        flush()
        front_group(*pend)

    def mm2_out(first):
        carry, started = [], []

        def emit(al, x, t0, t1):
            lanes = pl.ds(128 * t0, 128 * (t1 - t0))
            outv[al, :, lanes] = x.T.astype(bf16)
            cp = mk(outv.at[al, :, lanes], out_hbm.at[0, pl.ds(128 * al, 128), lanes], sem.at[SEM_OUT])
            cp.start()
            started.append(cp)

        def pin():
            outv[NB + zs[0], pl.ds(0, 16), pl.ds(0, 128)] = jnp.zeros((16, 128), bf16)
            return pltpu.bitcast(outv[NB + zs[0], pl.ds(0, 16), pl.ds(0, 128)], u32)

        for a in range(4):
            new = []

            def done(al, parts):
                x = _cat(parts)
                if al == 11:
                    emit(al, x[256:], 2, 5)
                elif al == 15:
                    emit(al, x[256:384], 2, 3)
                    emit(al, x[384:], 3, 5)
                else:
                    emit(al, x, 0, 5)
                new.append(pin)

            def early():
                feed(list(new), 1, 3 if a == 3 else 0)
                new.clear()
            plan = {1: [flush, P(feed, carry, 1)], 6: [early]}
            if a == 0:
                plan[0] = [P(feed, first, 6.5)]
            if a == 3:
                plan[5] = [early]
                plan[6] = [P(feed, [pin], 1, 3)]
            mm2_group(a, done, plan, (lambda al, parts: emit(al, _cat(parts)[:256], 0, 2)) if a == 3 else None)
            flush()
            carry = new
        wait(started)

    rstds = [{} for _ in range(4)]
    avail = []
    for n in range(NB + 2):
        if n in XWAIT:
            wait([cp for k, cp in enumerate(cp_x) if xsem[k] == xsem[n]])
            if n == XWAIT[-1]:
                start(cp_w[0] + cp_w[1], 0)
                start(cp_w1[0] + cp_w1[1], 1)
                wait(cp_b)
        dd = avail[:2 if n < NB else 1]
        del avail[:len(dd)]
        nd = len(dd) + (5 if n < NB else 0)
        if n >= 2:
            al = order16[n - 2]
            pieces = front_block(al, rstds[al % 4])
            if nd:
                feed(pieces, nd)
            else:
                run(pieces)
            if n % 4 == 1 and n < NB:
                avail.extend((al % 4, t) for t in range(5))
        if n < NB:
            xpose_in(order16[n])
        for a, t in dd:
            front_group(a, rstds[a], (t,))
        flush()
    for a, t in avail:
        front_group(a, rstds[a], (t,))
    front_group(3, rstds[3])

    bars[3].wait()
    mid({(False, 3): [P(wait, cp_w[0]), P(feed, wprep(0) + wprep(1), 54)],
         (True, 0): [flush, P(start, [cp_li], 0), P(start, cp_w1[2], 1), P(wait, cp_w[1]),
                     P(feed, wprep(2) + wprep(3), 42)],
         (True, 4): [flush]})
    wait([cp_li] + cp_w1[0])
    rem = back_mm1(0, P(wait, cp_w1[1]), lambda: (start(cp_w2, 1), wait(cp_w1[2])), P(wait, cp_w2))
    mm2_front(rem)
    bars[0].wait()
    mid()
    bars[1].wait()
    rem = back_mm1(1, bars[2].wait, lambda: None, lambda: None)
    mm2_out(rem)


@jax.jit
def pallas_interleave_layers__spectral_gfnet__mixer_token_mlp__prompt_kernel(
    A_x: jax.Array,
    A_w_r: jax.Array,
    A_w_i: jax.Array,
    B_x: jax.Array,
    B_w1: jax.Array,
    B_b1: jax.Array,
    B_w2: jax.Array,
    B_b2: jax.Array,
):
    del B_x
    lmat, tab = _constants()
    hbm = pl.BlockSpec(memory_space=pltpu.HBM)
    V = pltpu.VMEM
    return pl.pallas_call(
        _kernel,
        out_shape=jax.ShapeDtypeStruct((1, S, D), bf16),
        in_specs=[hbm] * 10,
        out_specs=hbm,
        scratch_shapes=[
            V((NB + 1, 128, D), bf16),
            V((2, D // 2 + 1, S), bf16),
            V((NB, F, 128), bf16),
            V((NB, F, 128), bf16),
            V((F,), bf16),
            V((NB, 128), bf16),
            V((10, 64, 128), u32),
            V((288, 128), f32),
            V((32, DH, 128), f32),
            V((7, DH, 2 * FQ + 128), f32),
            V((NB, 128), f32),
            V((NBAR, 8, 128), f32),
            pltpu.SMEM((8,), jnp.int32),
            pltpu.SemaphoreType.DMA((18 + NBAR,)),
            V((72, 48 * 128), u32),
            [V((33, 40, 128), u32)] * 4,
            [V((D + 80, 128), f32)] * NB,
            [V((DH + 8, 512), u32)] * 4,
            [V((4, 736, 128), f32)] * 4,
            [V((7, DH // 2 + 8, 256), u32)] * 4,
            [V((DH // 2 + 8, 256), u32)] * 2,
            V((50, DQ // 2, 256), u32),
            [[V((5, 72, 256), u32)] * 7] * 2,
            [V((5, 72, 256), u32)] * 7,
            [V((5, 72, 256), u32)] * 2,
            [V((50, 64, 256), u32)] * 3,
            [[V((FQ // 2 + 8, 7 * 128), u32)] * 7] * 4,
            [V((5, FR // 2 + 8, 256), u32)] * 4,
            V((50, DQ // 2, FQ), u32),
            V((DH // 2 + 8, 7 * 128), u32),
        ],
        compiler_params=pltpu.CompilerParams(vmem_limit_bytes=124 * 1024 * 1024, disable_semaphore_checks=True),
        name="gfmix",
    )(np.zeros((8,), np.int32), A_x, A_w_r.T, A_w_i.T, B_w1.T, B_b1, B_w2, B_b2.reshape(NB, 128), lmat, tab)
```
